```python
import os as _os
_os.environ.setdefault("JAX_PLATFORMS", "cpu")
import jax
import jax.numpy as jnp

def _softmax(x, axis=-1):
    return jax.nn.softmax(x, axis=axis)
def _gelu(x):
    return jax.nn.gelu(x, approximate=True)
def _silu(x):
    return jax.nn.silu(x)
def _sigmoid(x):
    return jax.nn.sigmoid(x)
def _layernorm(x, axis=-1, eps=1e-5):
    m = jnp.mean(x, axis=axis, keepdims=True)
    v = jnp.var(x, axis=axis, keepdims=True)
    return (x - m) / jnp.sqrt(v + eps)
def _scatter_add(tgt, idx, src, axis=0):
    return tgt.at[idx].add(src)
def _segment_sum(src, seg, n):
    return jax.ops.segment_sum(src, seg, n)
class _Rng:
    def __init__(self, key):
        self._k = key
    def _next(self):
        self._k, sub = jax.random.split(self._k)
        return sub
    def normal(self, shape):
        return jax.random.normal(self._next(), shape, dtype=jnp.bfloat16)
    def randint(self, lo, hi, shape):
        return jax.random.randint(self._next(), shape, lo, hi, dtype=jnp.int32)
    def uniform(self, shape, lo=0.0, hi=1.0):
        return jax.random.uniform(self._next(), shape, jnp.bfloat16, lo, hi)
    def permutation(self, n):
        return jax.random.permutation(self._next(), n)


kernel_name = 'concat_heads__gqa_block_cached__gqa_block_cached__near_ridge'

def setup_inputs():
    _rng = _Rng(jax.random.key(int.from_bytes(__import__("os").urandom(4), "little")))
    _w = (lambda a: (lambda t: t.astype(jnp.bfloat16) if jnp.issubdtype(t.dtype, jnp.floating) else t)(jnp.asarray(a)))
    def _A_setup():
        B, Sq, D = 8, 128, 576
        Hq, Hkv, Sk, Dh = 32, 16, 512, 128
        assert Hq % Hkv == 0, (Hq, Hkv)
        return {
            "x": _w((lambda *s: _rng.normal(s) * 0.8)(B, Sq, D)),
            "k_cache": _w((lambda *s: _rng.normal(s) * 0.8)(B, Hkv, Sk, Dh)),
            "v_cache": _w((lambda *s: _rng.normal(s) * 0.05)(B, Hkv, Sk, Dh)),
            "wq": _w((lambda *s: _rng.normal(s) * 0.8)(D, Hq * Dh) * (D ** -0.5)),
            "wo": _w((lambda *s: _rng.normal(s) * 0.05)(Hq * Dh, D) * ((Hq * Dh) ** -0.5)),
        }
    _A_in = _A_setup()

    def _B_setup():
        B, Sq, D = 8, 128, 576
        Hq, Hkv, Sk, Dh = 32, 16, 512, 128
        assert Hq % Hkv == 0, (Hq, Hkv)
        return {
            "x": _w((lambda *s: _rng.normal(s) * 0.8)(B, Sq, D)),
            "k_cache": _w((lambda *s: _rng.normal(s) * 0.8)(B, Hkv, Sk, Dh)),
            "v_cache": _w((lambda *s: _rng.normal(s) * 0.05)(B, Hkv, Sk, Dh)),
            "wq": _w((lambda *s: _rng.normal(s) * 0.8)(D, Hq * Dh) * (D ** -0.5)),
            "wo": _w((lambda *s: _rng.normal(s) * 0.05)(Hq * Dh, D) * ((Hq * Dh) ** -0.5)),
        }
    _B_in = _B_setup()

    return {
        "A_x": _A_in["x"],
        "A_k_cache": _A_in["k_cache"],
        "A_v_cache": _A_in["v_cache"],
        "A_wq": _A_in["wq"],
        "A_wo": _A_in["wo"],
        "B_x": _B_in["x"],
        "B_k_cache": _B_in["k_cache"],
        "B_v_cache": _B_in["v_cache"],
        "B_wq": _B_in["wq"],
        "B_wo": _B_in["wo"],
    }

def reference(A_x, A_k_cache, A_v_cache, A_wq, A_wo, B_x, B_k_cache, B_v_cache, B_wq, B_wo):
    def _A_ref(x, k_cache, v_cache, wq, wo):
        B, Sq, D = x.shape
        Hq, Dh = 32, 128
        Hkv = k_cache.shape[1]
        rep = Hq // Hkv
        q = (lambda x, *d: x.transpose(*d))((x @ wq).reshape(B, Sq, Hq, Dh), 0, 2, 1, 3)
        k = jnp.repeat(k_cache, rep, axis=1)
        v = jnp.repeat(v_cache, rep, axis=1)
        scores = jnp.einsum("bhqd,bhkd->bhqk", q, k) * (Dh ** -0.5)
        p = _softmax(scores, axis=-1)
        o = jnp.einsum("bhqk,bhkd->bhqd", p, v)
        return (lambda x, *d: x.transpose(*d))(o, 0, 2, 1, 3).reshape(B, Sq, Hq * Dh) @ wo

    def _B_ref(x, k_cache, v_cache, wq, wo):
        B, Sq, D = x.shape
        Hq, Dh = 32, 128
        Hkv = k_cache.shape[1]
        rep = Hq // Hkv
        q = (lambda x, *d: x.transpose(*d))((x @ wq).reshape(B, Sq, Hq, Dh), 0, 2, 1, 3)
        k = jnp.repeat(k_cache, rep, axis=1)
        v = jnp.repeat(v_cache, rep, axis=1)
        scores = jnp.einsum("bhqd,bhkd->bhqk", q, k) * (Dh ** -0.5)
        p = _softmax(scores, axis=-1)
        o = jnp.einsum("bhqk,bhkd->bhqd", p, v)
        return (lambda x, *d: x.transpose(*d))(o, 0, 2, 1, 3).reshape(B, Sq, Hq * Dh) @ wo

    a = _A_ref(A_x, A_k_cache, A_v_cache, A_wq, A_wo)
    b = _B_ref(B_x, B_k_cache, B_v_cache, B_wq, B_wo)
    return jnp.concatenate([a, b], axis=-1)
```

```python
import math

import jax
import jax.numpy as jnp
import jax.experimental.pallas as pl
import jax.experimental.pallas.tpu as pltpu

B, SQ, D = 8, 128, 576
HQ, HKV, SK, DH = 32, 16, 512, 128
REP = HQ // HKV
HD = REP * DH
QSCALE = (DH ** -0.5) * math.log2(math.e)
BF = jnp.bfloat16
F32 = jnp.float32
NT = (((1,), (1,)), ((), ()))

GQ = 4
CW = GQ * HD
NQ = HKV // GQ
RING = 2
GROUPS = (8, 6, 2)
STARTS = tuple(sum(GROUPS[:g]) for g in range(len(GROUPS)))
GL = GROUPS[-1]


def _kernel(ax, ak, av, awq, awo, bx, bk, bv, bwq, bwo, out_hbm,
            xt_v, x_v, wq_v, wo_v, kbuf, vbuf, q_scr, o_scr, acc, ostage,
            sem_x, sem_wq, sem_wo, sem_kv, sem_out):
    xs = (ax, bx)
    ks = (ak, bk)
    vs = (av, bv)
    wqs = (awq, bwq)
    wos = (awo, bwo)

    def x_cp(blk):
        return pltpu.make_async_copy(xs[blk], xt_v.at[blk], sem_x.at[blk])

    def wq_cp(blk, j):
        c0 = j * CW if isinstance(j, int) else pl.multiple_of(j * CW, CW)
        return pltpu.make_async_copy(wqs[blk].at[:, pl.ds(c0, CW)],
                                     wq_v.at[blk, :, pl.ds(c0, CW)], sem_wq.at[blk, j])

    def wo_cp(blk):
        return pltpu.make_async_copy(wos[blk], wo_v.at[blk], sem_wo.at[blk])

    def kv_cps(b):
        slot = b % RING
        cps = []
        for blk in range(2):
            cps.append(pltpu.make_async_copy(ks[blk].at[b], kbuf.at[slot, blk],
                                             sem_kv.at[slot, 2 * blk]))
            cps.append(pltpu.make_async_copy(vs[blk].at[b], vbuf.at[slot, blk],
                                             sem_kv.at[slot, 2 * blk + 1]))
        return cps

    def out_cp(b):
        return pltpu.make_async_copy(ostage.at[b], out_hbm.at[b], sem_out.at[b])

    def qproj(blk, j):
        c0 = j * CW if isinstance(j, int) else pl.multiple_of(j * CW, CW)
        q = jnp.dot(x_v[blk], wq_v[blk, :, pl.ds(c0, CW)], preferred_element_type=F32)
        q = (q * QSCALE).astype(BF).reshape(B, SQ, CW)
        for g in range(GQ):
            for r in range(REP):
                c = (g * REP + r) * DH
                q_scr[blk, j * GQ + g, :, r * SQ:(r + 1) * SQ, :] = q[:, :, c:c + DH]

    x_cp(0).start()
    wq_cp(0, 0).start()
    x_cp(0).wait()
    wq_cp(0, 1).start()
    x_cp(1).start()

    def xpose_a(b, _):
        r0 = pl.multiple_of(b * SQ, SQ)
        x_v[0, pl.ds(r0, SQ), :] = xt_v[0, b].T
        return 0
    jax.lax.fori_loop(0, B, xpose_a, 0)

    def p1a(j, _):
        @pl.when(j + 2 < NQ)
        def _():
            wq_cp(0, j + 2).start()

        @pl.when(j + 2 >= NQ)
        def _():
            wq_cp(1, j + 2 - NQ).start()
        wq_cp(0, j).wait()
        qproj(0, j)
        return 0
    jax.lax.fori_loop(0, NQ - 1, p1a, 0)

    wq_cp(1, 1).start()
    wo_cp(0).start()
    wo_cp(1).start()
    wq_cp(0, NQ - 1).wait()
    x_cp(1).wait()
    for b in range(B):
        x_v[1, b * SQ:(b + 1) * SQ, :] = xt_v[1, b].T
    qproj(0, NQ - 1)

    def p1b(j, _):
        @pl.when(j + 2 < NQ)
        def _():
            wq_cp(1, j + 2).start()

        @pl.when(j == 0)
        def _():
            for cp in kv_cps(0):
                cp.start()
        wq_cp(1, j).wait()
        qproj(1, j)
        return 0
    jax.lax.fori_loop(0, NQ, p1b, 0)

    acc[1] = jnp.zeros(acc.shape[1:], F32)
    o_scr[...] = jnp.zeros_like(o_scr)
    wo_cp(0).wait()
    wo_cp(1).wait()

    def scores_softmax(b, blk, j):
        slot = b % RING
        s = jax.lax.dot_general(q_scr[blk, j, b], kbuf[slot, blk, j], NT,
                                preferred_element_type=F32)
        m = jnp.max(s, axis=-1, keepdims=True)
        p = jnp.exp2(s - m)
        l = jnp.sum(p, axis=-1, keepdims=True)
        return p.astype(BF), l

    def pv(b, blk, j, p, l):
        slot = b % RING
        o = jnp.dot(p, vbuf[slot, blk, j], preferred_element_type=F32)
        r = pl.reciprocal(l, approx=True)
        r = r * (2.0 - l * r)
        o = (o * r).astype(BF)
        return [o[:SQ], o[SQ:]]

    def outproj(par, blk, h0, oc, first):
        c0 = h0 * HD
        res = jax.lax.dot_general(wo_v[blk, :, c0:c0 + oc.shape[1]], oc, NT,
                                  preferred_element_type=F32)
        if first:
            acc[par, blk * D:(blk + 1) * D, :] = res
        else:
            acc[par, blk * D:(blk + 1) * D, :] += res

    def finish_prev(par_prev, slot):
        for blk in range(2):
            outproj(par_prev, blk, HKV - GL, o_scr[blk], False)
        ostage[slot] = acc[par_prev].T.astype(BF)

    n_g = len(GROUPS)

    def p2(b, _):
        @pl.when(b + 1 < B)
        def _():
            for cp in kv_cps(b + 1):
                cp.start()
        for cp in kv_cps(b):
            cp.wait()
        par = b % 2
        finish_prev(1 - par, jnp.where(b > 0, b - 1, B))

        pend = {0: [], 1: []}
        cur = {0: [], 1: []}
        gi = 0
        st = {0: scores_softmax(b, 0, 0), 1: scores_softmax(b, 1, 0)}
        for j in range(HKV):
            for blk in range(2):
                p, l = st[blk]
                if j + 1 < HKV:
                    st[blk] = scores_softmax(b, blk, j + 1)
                cur[blk] += pv(b, blk, j, p, l)
                if j + 1 == STARTS[gi] + GROUPS[gi]:
                    pend[blk].append((gi, cur[blk]))
                    cur[blk] = []
                while len(pend[blk]) > 1 and pend[blk][0][0] < n_g - 1:
                    g, parts = pend[blk].pop(0)
                    outproj(par, blk, STARTS[g], jnp.concatenate(parts, axis=1), g == 0)
            if j + 1 == STARTS[gi] + GROUPS[gi]:
                gi += 1
        for blk in range(2):
            for g, parts in pend[blk]:
                if g < n_g - 1:
                    outproj(par, blk, STARTS[g], jnp.concatenate(parts, axis=1), g == 0)
                else:
                    o_scr[blk] = jnp.concatenate(parts, axis=1)

        @pl.when(b > 0)
        def _():
            out_cp(b - 1).start()
        return 0
    jax.lax.fori_loop(0, B, p2, 0)

    finish_prev((B - 1) % 2, B - 1)
    out_cp(B - 1).start()
    for b in range(B):
        out_cp(b).wait()


@jax.jit
def pallas_concat_heads__gqa_block_cached__gqa_block_cached__near_ridge_kernel(
    A_x: jax.Array,
    A_k_cache: jax.Array,
    A_v_cache: jax.Array,
    A_wq: jax.Array,
    A_wo: jax.Array,
    B_x: jax.Array,
    B_k_cache: jax.Array,
    B_v_cache: jax.Array,
    B_wq: jax.Array,
    B_wo: jax.Array,
):
    hbm = pl.BlockSpec(memory_space=pltpu.HBM)
    return pl.pallas_call(
        _kernel,
        in_specs=[hbm] * 10,
        out_specs=hbm,
        out_shape=jax.ShapeDtypeStruct((B, SQ, 2 * D), BF),
        scratch_shapes=[
            pltpu.VMEM((2, B, D, SQ), BF),
            pltpu.VMEM((2, B * SQ, D), BF),
            pltpu.VMEM((2, D, HQ * DH), BF),
            pltpu.VMEM((2, D, HQ * DH), BF),
            pltpu.VMEM((RING, 2, HKV, SK, DH), BF),
            pltpu.VMEM((RING, 2, HKV, SK, DH), BF),
            pltpu.VMEM((2, HKV, B, REP * SQ, DH), BF),
            pltpu.VMEM((2, SQ, GL * HD), BF),
            pltpu.VMEM((2, 2 * D, SQ), F32),
            pltpu.VMEM((B + 1, SQ, 2 * D), BF),
            pltpu.SemaphoreType.DMA((2,)),
            pltpu.SemaphoreType.DMA((2, NQ)),
            pltpu.SemaphoreType.DMA((2,)),
            pltpu.SemaphoreType.DMA((RING, 4)),
            pltpu.SemaphoreType.DMA((B,)),
        ],
        compiler_params=pltpu.CompilerParams(vmem_limit_bytes=100 * 1024 * 1024),
    )(A_x.transpose(0, 2, 1), A_k_cache, A_v_cache, A_wq, A_wo.T,
      B_x.transpose(0, 2, 1), B_k_cache, B_v_cache, B_wq, B_wo.T)
```
